```python
import os as _os
_os.environ.setdefault("JAX_PLATFORMS", "cpu")
import jax
import jax.numpy as jnp

def _softmax(x, axis=-1):
    return jax.nn.softmax(x, axis=axis)
def _gelu(x):
    return jax.nn.gelu(x, approximate=True)
def _silu(x):
    return jax.nn.silu(x)
def _sigmoid(x):
    return jax.nn.sigmoid(x)
def _layernorm(x, axis=-1, eps=1e-5):
    m = jnp.mean(x, axis=axis, keepdims=True)
    v = jnp.var(x, axis=axis, keepdims=True)
    return (x - m) / jnp.sqrt(v + eps)
def _scatter_add(tgt, idx, src, axis=0):
    return tgt.at[idx].add(src)
def _segment_sum(src, seg, n):
    return jax.ops.segment_sum(src, seg, n)
class _Rng:
    def __init__(self, key):
        self._k = key
    def _next(self):
        self._k, sub = jax.random.split(self._k)
        return sub
    def normal(self, shape):
        return jax.random.normal(self._next(), shape, dtype=jnp.bfloat16)
    def randint(self, lo, hi, shape):
        return jax.random.randint(self._next(), shape, lo, hi, dtype=jnp.int32)
    def uniform(self, shape, lo=0.0, hi=1.0):
        return jax.random.uniform(self._next(), shape, jnp.bfloat16, lo, hi)
    def permutation(self, n):
        return jax.random.permutation(self._next(), n)


kernel_name = 'standalone__grn__sampling'

def setup_inputs():
    _rng = _Rng(jax.random.key(int.from_bytes(__import__("os").urandom(4), "little")))
    _w = (lambda a: (lambda t: t.astype(jnp.bfloat16) if jnp.issubdtype(t.dtype, jnp.floating) else t)(jnp.asarray(a)))
    B, S, D = 512, 32, 640
    return {
        "x": _w((lambda *s: _rng.normal(s) * 0.05)(B, S, D)),
        "g": _w((lambda *s: _rng.normal(s) * 0.1)(D) * 0.1),
        "b": _w((lambda *s: _rng.normal(s) * 0.1)(D) * 0.1),
    }

def reference(x, g, b):
    gx = jnp.sqrt((x * x).sum(axis=-2, keepdims=True))
    nx = gx / (gx.mean(axis=-1, keepdims=True) + 1e-6)
    return g * (x * nx) + b + x
```

```python
import jax
import jax.numpy as jnp
from jax import lax
import jax.experimental.pallas as pl
import jax.experimental.pallas.tpu as pltpu

_EPS = 1e-6


@jax.jit
def pallas_standalone__grn__sampling_kernel(
    x: jax.Array,
    g: jax.Array,
    b: jax.Array,
):
    B, S, D = x.shape
    Q = 8
    N = B // Q
    L = 4
    NS = 8
    W0 = 2
    WN = 4
    assert B % Q == 0 and 0 <= W0 < L < NS and WN <= N - L

    def kern(x_hbm, g_hbm, b_hbm, o_hbm, xbuf, obuf, gbuf, bbuf, scr, rsem, wsem):
        def rd1(j, q):
            pltpu.make_async_copy(
                x_hbm.at[q, j], xbuf.at[j, q], rsem.at[j & (NS - 1)]
            ).start(priority=q % 2)

        def rd_wait(j):
            pltpu.make_async_copy(xbuf.at[j], xbuf.at[j], rsem.at[j & (NS - 1)]).wait()

        def wr_start(j):
            pltpu.make_async_copy(obuf.at[j], o_hbm.at[:, j], wsem).start()

        for q in range(Q):
            rd1(0, q)
        cg = pltpu.make_async_copy(g_hbm, gbuf, wsem)
        cg.start()
        cb = pltpu.make_async_copy(b_hbm, bbuf, wsem)
        cb.start()

        def pro(j, c):
            for q in range(Q):
                rd1(j, q)
            return c

        lax.fori_loop(1, L, pro, 0)
        cg.wait()
        cb.wait()
        gv = gbuf[...].astype(jnp.float32).reshape(1, D)
        bv = bbuf[...].astype(jnp.float32).reshape(1, D)

        def comp(j, issue):
            for q in range(Q):
                xv = xbuf[j, q].astype(jnp.float32)
                scr[pl.ds(q, 1), :] = jnp.sum(xv * xv, axis=0, keepdims=True)
                if issue and q % 2 == 1:
                    rd1(j + L, q // 2)
            gx = jnp.sqrt(scr[...])
            m = jnp.mean(gx, axis=-1, keepdims=True)
            nx = gx / (m + _EPS)
            scr[...] = gv * nx + 1.0
            for q in range(Q):
                xv = xbuf[j, q].astype(jnp.float32)
                s = scr[pl.ds(q, 1), :]
                obuf[j, q] = (xv * s + bv).astype(obuf.dtype)
                if issue and q % 2 == 1:
                    rd1(j + L, Q // 2 + q // 2)

        def body(j, c):
            rd_wait(j)
            comp(j, True)
            return c

        lax.fori_loop(0, N - L, body, 0)

        def body2(j, c):
            rd_wait(j)

            @pl.when(j == N - W0 - 1)
            def _():
                for t in range(WN):
                    wr_start(t)

            comp(j, False)
            return c

        lax.fori_loop(N - L, N, body2, 0)

        def wbody(j, c):
            wr_start(j)
            return c

        lax.fori_loop(WN, N, wbody, 0)
        pltpu.make_async_copy(obuf, obuf, wsem).wait()

    xr = x.reshape(Q, N, S, D)
    out = pl.pallas_call(
        kern,
        in_specs=[pl.BlockSpec(memory_space=pl.ANY)] * 3,
        out_specs=pl.BlockSpec(memory_space=pl.ANY),
        out_shape=jax.ShapeDtypeStruct(xr.shape, x.dtype),
        scratch_shapes=[
            pltpu.VMEM((N, Q, S, D), x.dtype),
            pltpu.VMEM((N, Q, S, D), x.dtype),
            pltpu.VMEM((D,), g.dtype),
            pltpu.VMEM((D,), b.dtype),
            pltpu.VMEM((Q, D), jnp.float32),
            pltpu.SemaphoreType.DMA((NS,)),
            pltpu.SemaphoreType.DMA(()),
        ],
        compiler_params=pltpu.CompilerParams(
            vmem_limit_bytes=64 * 1024 * 1024,
            disable_bounds_checks=True,
        ),
    )(xr, g, b)
    return out.reshape(B, S, D)
```

```python
import jax
import jax.numpy as jnp
from jax import lax
import jax.experimental.pallas as pl
import jax.experimental.pallas.tpu as pltpu

_EPS = 1e-6


@jax.jit
def pallas_standalone__grn__sampling_kernel(
    x: jax.Array,
    g: jax.Array,
    b: jax.Array,
):
    B, S, D = x.shape
    Q = 8
    H = Q // 2
    N = B // Q
    C = D // 128
    R = S // 8
    L0 = 3
    L1 = 9
    NS = 16
    W0 = 2
    WN = 16
    assert B % Q == 0 and S % 8 == 0 and D % 128 == 0
    assert 0 <= W0 <= L0 <= L1 and L1 + 1 < NS and WN <= N - L1 - 2

    def tree_sum(vals):
        vals = list(vals)
        while len(vals) > 1:
            nxt = [vals[i] + vals[i + 1] for i in range(0, len(vals) - 1, 2)]
            if len(vals) % 2:
                nxt.append(vals[-1])
            vals = nxt
        return vals[0]

    def kern(x_hbm, g_hbm, b_hbm, o_hbm, xbuf, obuf, gbuf, bbuf, acc, sc, gb8, wsem):
        def wr_start(j, carry):
            pltpu.make_async_copy(obuf.at[j], o_hbm.at[:, j], wsem).start()
            return carry

        def main(rsem):
            def rd(j, q):
                pltpu.make_async_copy(
                    x_hbm.at[q, j], xbuf.at[j, q], rsem.at[j & (NS - 1)]
                ).start(priority=q % 2)

            def rd_wait(j):
                pltpu.make_async_copy(
                    xbuf.at[j], xbuf.at[j], rsem.at[j & (NS - 1)]
                ).wait()

            for q in range(Q):
                rd(0, q)
            cg = pltpu.make_async_copy(g_hbm, gbuf, wsem)
            cb = pltpu.make_async_copy(b_hbm, bbuf, wsem)
            cg.start()
            cb.start()

            def pro_p1(j, carry):
                for q in range(1, Q, 2):
                    rd(j, q)
                return carry

            lax.fori_loop(1, L1 - L0 + 1, pro_p1, 0)

            def pro_both(j, carry):
                for h in range(H):
                    rd(j + L1 - L0, 2 * h + 1)
                    rd(j, 2 * h)
                return carry

            lax.fori_loop(1, L0 + 1, pro_both, 0)
            cg.wait()
            cb.wait()
            gb8[0] = jnp.broadcast_to(gbuf[...].astype(jnp.float32).reshape(1, D), (8, D))
            gb8[1] = jnp.broadcast_to(bbuf[...].astype(jnp.float32).reshape(1, D), (8, D))

            def sumsq(j, q, slot):
                xv = xbuf[j, q].astype(jnp.float32)
                x2 = xv * xv
                p = tree_sum(x2[r * 8:(r + 1) * 8] for r in range(R))
                for c in range(C):
                    acc[slot, c, pl.ds(q, 8, stride=Q), :] = p[:, c * 128:(c + 1) * 128]

            def stats(slot):
                gx = [
                    jnp.sqrt(tree_sum(acc[slot, c, pl.ds(s * Q, Q), :] for s in range(8)))
                    for c in range(C)
                ]
                mean = jnp.sum(tree_sum(gx), axis=-1, keepdims=True) * (1.0 / D)
                inv = 1.0 / (mean + _EPS)
                for c in range(C):
                    sc[slot, c] = (gx[c] * inv) * gb8[0, :, c * 128:(c + 1) * 128] + 1.0

            def scale(j, q, slot):
                xv = xbuf[j, q].astype(jnp.float32)
                s8 = jnp.concatenate(
                    [jnp.broadcast_to(sc[slot, c, pl.ds(q, 1), :], (8, 128)) for c in range(C)],
                    axis=1,
                )
                b8 = gb8[1]
                out = jnp.concatenate(
                    [xv[r * 8:(r + 1) * 8] * s8 + b8 for r in range(R)], axis=0
                )
                obuf[j, q] = out.astype(obuf.dtype)

            def work(j, slot, p0, p1, last=False):
                def issue(k):
                    if k % 2 == 0 and p0:
                        rd(j + 1 + L0, k)
                    if k % 2 == 1 and p1:
                        rd(j + 1 + L1, k)

                stats(slot)
                if not last:
                    for q in range(Q):
                        sumsq(j + 1, q, 1 - slot)
                        if q % 2 == 1:
                            issue(q // 2)
                for q in range(Q):
                    scale(j, q, slot)
                    if q % 2 == 1:
                        issue(H + q // 2)

            def run(ja, jb, p0, p1):
                j = ja
                if j < jb and j % 2:
                    rd_wait(j + 1)
                    work(j, 1, p0, p1)
                    j += 1
                npair = (jb - j) // 2
                if npair:
                    def body(i, carry):
                        for k in range(2):
                            rd_wait(2 * i + k + 1)
                            work(2 * i + k, k, p0, p1)
                        return carry

                    lax.fori_loop(j // 2, j // 2 + npair, body, 0)
                    j += 2 * npair
                if j < jb:
                    rd_wait(j + 1)
                    work(j, 0, p0, p1)

            rd_wait(0)
            for q in range(Q):
                sumsq(0, q, 0)
            n1 = N - L1 - 1
            n0 = N - L0 - 1
            gt = N - W0 - 1
            run(0, n1, True, True)
            run(n1, n0, True, False)

            for gi in range(n0 + 1, gt + 1):
                rd_wait(gi)
            lax.fori_loop(0, WN, wr_start, 0)
            for j in range(n0, N):
                if gt < j + 1 < N:
                    rd_wait(j + 1)
                work(j, j % 2, False, False, last=(j == N - 1))
            lax.fori_loop(WN, N, wr_start, 0)

        pl.run_scoped(main, pltpu.SemaphoreType.DMA((NS,)))
        pltpu.make_async_copy(o_hbm, o_hbm, wsem).wait()

    xr = x.reshape(Q, N, S, D)
    out = pl.pallas_call(
        kern,
        in_specs=[pl.BlockSpec(memory_space=pl.ANY)] * 3,
        out_specs=pl.BlockSpec(memory_space=pl.ANY),
        out_shape=jax.ShapeDtypeStruct(xr.shape, x.dtype),
        scratch_shapes=[
            pltpu.VMEM((N, Q, S, D), x.dtype),
            pltpu.VMEM((N, Q, S, D), x.dtype),
            pltpu.VMEM((D,), g.dtype),
            pltpu.VMEM((D,), b.dtype),
            pltpu.VMEM((2, C, 8 * Q + 8, 128), jnp.float32),
            pltpu.VMEM((2, C, Q, 128), jnp.float32),
            pltpu.VMEM((2, 8, D), jnp.float32),
            pltpu.SemaphoreType.DMA(()),
        ],
        compiler_params=pltpu.CompilerParams(vmem_limit_bytes=64 * 1024 * 1024),
    )(xr, g, b)
    return out.reshape(B, S, D)
```
